```python
import os as _os
_os.environ.setdefault("JAX_PLATFORMS", "cpu")
import jax
import jax.numpy as jnp

def _softmax(x, axis=-1):
    return jax.nn.softmax(x, axis=axis)
def _gelu(x):
    return jax.nn.gelu(x, approximate=True)
def _silu(x):
    return jax.nn.silu(x)
def _sigmoid(x):
    return jax.nn.sigmoid(x)
def _layernorm(x, axis=-1, eps=1e-5):
    m = jnp.mean(x, axis=axis, keepdims=True)
    v = jnp.var(x, axis=axis, keepdims=True)
    return (x - m) / jnp.sqrt(v + eps)
def _scatter_add(tgt, idx, src, axis=0):
    return tgt.at[idx].add(src)
def _segment_sum(src, seg, n):
    return jax.ops.segment_sum(src, seg, n)
class _Rng:
    def __init__(self, key):
        self._k = key
    def _next(self):
        self._k, sub = jax.random.split(self._k)
        return sub
    def normal(self, shape):
        return jax.random.normal(self._next(), shape, dtype=jnp.bfloat16)
    def randint(self, lo, hi, shape):
        return jax.random.randint(self._next(), shape, lo, hi, dtype=jnp.int32)
    def uniform(self, shape, lo=0.0, hi=1.0):
        return jax.random.uniform(self._next(), shape, jnp.bfloat16, lo, hi)
    def permutation(self, n):
        return jax.random.permutation(self._next(), n)


kernel_name = 'recurrent_scan__ssm_conv_s4__mixer_s_mlp__prompt'

def setup_inputs():
    _rng = _Rng(jax.random.key(int.from_bytes(__import__("os").urandom(4), "little")))
    _w = (lambda a: (lambda t: t.astype(jnp.bfloat16) if jnp.issubdtype(t.dtype, jnp.floating) else t)(jnp.asarray(a)))
    def _A_setup():
        B, L, D, N = 1, 2048, 512, 128
        A_re = -jnp.exp((lambda *s: _rng.normal(s) * 0.1)(D, N))
        A_im = jnp.pi * (lambda *s: _rng.normal(s) * 0.1)(D, N)
        B_re = (lambda *s: _rng.normal(s) * 0.1)(D, N)
        B_im = (lambda *s: _rng.normal(s) * 0.1)(D, N)
        C_re = (lambda *s: _rng.normal(s) * 0.1)(D, N)
        C_im = (lambda *s: _rng.normal(s) * 0.1)(D, N)
        log_dt = (lambda *s: _rng.normal(s) * 0.1)(D) * 0.5 - 4.0
        Dskip = (lambda *s: _rng.normal(s) * 0.05)(D)
        return {
            "u": _w((lambda *s: _rng.normal(s) * 0.05)(B, L, D)),
            "A_re": _w(A_re),
            "A_im": _w(A_im),
            "B_re": _w(B_re),
            "B_im": _w(B_im),
            "C_re": _w(C_re),
            "C_im": _w(C_im),
            "log_dt": _w(log_dt),
            "Dskip": _w(Dskip),
        }
    _A_in = _A_setup()

    def _B_setup():
        B, S, D, F = 1, 2048, 512, 1376
        return {
            "x":  _w((lambda *s: _rng.normal(s) * 0.05)(B, S, D)),
            "w1": _w((lambda *s: _rng.normal(s) * 0.8)(D, D) * (D ** -0.5)),
            "w2": _w((lambda *s: _rng.normal(s) * 0.8)(D, D) * (D ** -0.5)),
            "w3": _w((lambda *s: _rng.normal(s) * 0.8)(D, F) * (D ** -0.5)),
            "w4": _w((lambda *s: _rng.normal(s) * 0.8)(F, D) * (F ** -0.5)),
        }
    _B_in = _B_setup()

    return {
        "A_u": _A_in["u"],
        "A_A_re": _A_in["A_re"],
        "A_A_im": _A_in["A_im"],
        "A_B_re": _A_in["B_re"],
        "A_B_im": _A_in["B_im"],
        "A_C_re": _A_in["C_re"],
        "A_C_im": _A_in["C_im"],
        "A_log_dt": _A_in["log_dt"],
        "A_Dskip": _A_in["Dskip"],
        "B_x": _B_in["x"],
        "B_w1": _B_in["w1"],
        "B_w2": _B_in["w2"],
        "B_w3": _B_in["w3"],
        "B_w4": _B_in["w4"],
    }

def reference(A_u, A_A_re, A_A_im, A_B_re, A_B_im, A_C_re, A_C_im, A_log_dt, A_Dskip, B_x, B_w1, B_w2, B_w3, B_w4):
    def _A_ref(u, A_re, A_im, B_re, B_im, C_re, C_im, log_dt, Dskip):
        Bsz, L, D = u.shape
        dt = jnp.exp(log_dt)[:, None]
        A = A_re + 1j * A_im
        Bc = B_re + 1j * B_im
        Cc = C_re + 1j * C_im
        logdA = dt * A
        dB = dt * Bc
        l = (lambda x, dt: x.astype(dt))(jnp.arange(L), A_re.dtype)
        P = jnp.exp(logdA[:, :, None] * l[None, None, :])
        K = jnp.einsum("dn,dnl,dn->dl", Cc, P, dB).real
        L2 = 2 * L
        Kp = jnp.pad(K, ((0, 0), (0, L)))
        up = (lambda x, *d: x.transpose(*d))(u, 0, 2, 1)
        up = jnp.pad(up, ((0, 0), (0, 0), (0, L)))
        Kf = (lambda x, axes=(-2,-1): jnp.fft.rfft2(x.astype(jnp.float32), axes=axes))(Kp[:, None, :], axes=(-2, -1))
        Uf = (lambda x, axes=(-2,-1): jnp.fft.rfft2(x.astype(jnp.float32), axes=axes))(up[:, :, None, :], axes=(-2, -1))
        Yf = Uf * Kf[None, :, :, :]
        y = (lambda x, s, axes=(-2,-1): jnp.fft.irfft2(x, s=s, axes=axes).astype(jnp.bfloat16))(Yf, (1, L2), axes=(-2, -1))[:, :, 0, :L]
        y = (lambda x, *d: x.transpose(*d))(y, 0, 2, 1) + u * Dskip[None, None, :]
        return y

    def _B_ref(x, w1, w2, w3, w4):
        B, S, D = x.shape
        h = _gelu(_layernorm(x, axis=-1) @ w1)
        c = D // 4
        g0 = jnp.pad(h[:, :, 0*c:1*c], ((0, 0), (1, 0), (0, 0)))[:, :S, :]
        g1 = jnp.pad(h[:, :, 1*c:2*c], ((0, 0), (0, 1), (0, 0)))[:, 1:, :]
        g2 = jnp.pad(h[:, :, 2*c:3*c], ((0, 0), (2, 0), (0, 0)))[:, :S, :]
        g3 = jnp.pad(h[:, :, 3*c:   ], ((0, 0), (0, 2), (0, 0)))[:, 2:, :]
        hs = jnp.concatenate([g0, g1, g2, g3], axis=-1) @ w2
        x1 = x + hs
        h2 = _gelu(_layernorm(x1, axis=-1) @ w3) @ w4
        return x1 + h2

    x = A_u
    xn = _layernorm(x, axis=-1)
    s = _A_ref(xn, A_A_re, A_A_im, A_B_re, A_B_im, A_C_re, A_C_im, A_log_dt, A_Dskip)
    g = _silu(_B_ref(xn, B_w1, B_w2, B_w3, B_w4))
    return x + s * g
```

```python
import numpy as np
import jax
import jax.numpy as jnp
from jax import lax
import jax.experimental.pallas as pl
import jax.experimental.pallas.tpu as pltpu

L = 2048
D = 512
N = 128
F = 1376
T = 128
NB = L // T
PAD = 16
EPS = 1e-5
GRP = 8

_ALPHA = (
    [j for j in range(8)]
    + [128 + j for j in range(8)]
    + [256 + 2 * j for j in range(4)] + [384 + 2 * j for j in range(4)]
    + [512 + 128 * i + e for i in range(4) for e in (0, 4)]
    + [1024 + 128 * j for j in range(8)]
    + [2048]
)
_NA = len(_ALPHA)
_NSLAB = 6
_NBETA = 16


def _build_tables():
    r_of_l = np.arange(L, dtype=np.float32).astype(jnp.bfloat16).astype(np.int64)
    pos = {}
    for a, al in enumerate(_ALPHA):
        for b in range(_NBETA):
            pos.setdefault(al + 8 * b, (a // 8, (8 * b + a % 8 + 7) % 128))
    k = np.arange(T, dtype=np.float64)
    theta = np.pi * (2 * k + 1) / (2 * T)
    ll = np.arange(T, dtype=np.float64)
    zc = np.exp(-1j * theta[:, None] * ll[None, :])
    s = 1j * np.where(np.arange(T) % 2 == 0, 1.0, -1.0)
    ffwd = np.concatenate([zc.real, zc.imag], axis=0)
    finv = np.concatenate([np.cos(theta[None, :] * ll[:, None]),
                           -np.sin(theta[None, :] * ll[:, None])], axis=1) / T
    mats, plan = [], []
    for m in range(NB):
        acc = np.zeros((_NSLAB, T, 128), dtype=np.complex128)
        for l in range(T):
            sl, lane = pos[int(r_of_l[T * m + l])]
            acc[sl, :, lane] += zc[:, l]
            if m > 0:
                sl, lane = pos[int(r_of_l[T * (m - 1) + l])]
                acc[sl, :, lane] += s * zc[:, l]
        for sl in range(_NSLAB):
            if np.any(acc[sl] != 0):
                plan.append((m, sl))
                mats.append(np.concatenate([acc[sl].real, acc[sl].imag], axis=0))
    return (ffwd.astype(np.float32), finv.astype(np.float32),
            np.stack(mats).astype(np.float32), tuple(plan))


_FFWD, _FINV, _FSEL, _PLAN = _build_tables()
_NSEL = len(_PLAN)


def _cmul(a, b):
    return (a[0] * b[0] - a[1] * b[1], a[0] * b[1] + a[1] * b[0])


def _ln(x):
    m = jnp.mean(x, axis=-1, keepdims=True)
    xc = x - m
    v = jnp.mean(xc * xc, axis=-1, keepdims=True)
    return xc * lax.rsqrt(v + EPS)


def _gelu(x):
    return 0.5 * x * (1.0 + jnp.tanh(0.7978845608028654 * (x + 0.044715 * (x * x * x))))


def _bf(x):
    return x.astype(jnp.bfloat16)


def _kernel(u_hbm, are_ref, aim_ref, bre_ref, bim_ref, cre_ref, cim_ref,
            ldt_ref, dskip_ref, w1_hbm, w2_hbm, w3_hbm, w4_hbm,
            ffwd_ref, finv_ref, fsel_hbm,
            out_hbm,
            u_v, w1_v, w2_v, w3_v, w4_v, fsel_v, gt_v, kf_v, uf_v, acc_v, out_v,
            in_sems, out_sems):
    f32 = jnp.float32

    copies = [
        pltpu.make_async_copy(fsel_hbm, fsel_v, in_sems.at[0]),
        pltpu.make_async_copy(u_hbm, u_v.at[pl.ds(PAD, L)], in_sems.at[1]),
        pltpu.make_async_copy(w1_hbm, w1_v, in_sems.at[2]),
        pltpu.make_async_copy(w2_hbm, w2_v, in_sems.at[3]),
        pltpu.make_async_copy(w3_hbm, w3_v, in_sems.at[4]),
        pltpu.make_async_copy(w4_hbm, w4_v, in_sems.at[5]),
    ]
    for c in copies:
        c.start()

    u_v[pl.ds(0, PAD), :] = jnp.zeros((PAD, D), jnp.bfloat16)
    u_v[pl.ds(PAD + L, PAD), :] = jnp.zeros((PAD, D), jnp.bfloat16)

    def kgen_rows(row0, nrows):
        sl = pl.ds(row0, nrows)
        dt = jnp.exp(ldt_ref[sl, :].astype(f32)).astype(jnp.bfloat16).astype(f32)
        lr = dt * are_ref[sl, :].astype(f32)
        li = dt * aim_ref[sl, :].astype(f32)
        mag = jnp.exp(lr)
        lam = (mag * jnp.cos(li), mag * jnp.sin(li))
        db = (dt * bre_ref[sl, :].astype(f32), dt * bim_ref[sl, :].astype(f32))
        w = _cmul((cre_ref[sl, :].astype(f32), cim_ref[sl, :].astype(f32)), db)
        one = (jnp.ones_like(lr), jnp.zeros_like(lr))
        small = [one, lam]
        for _ in range(2, 9):
            small.append(_cmul(small[-1], lam))
        lam8 = small[8]
        lam128 = lam8
        for _ in range(4):
            lam128 = _cmul(lam128, lam128)
        wj = [w]
        for _ in range(1, 17):
            wj.append(_cmul(wj[-1], lam128))
        xs = []
        for al in _ALPHA:
            j, e = al // 128, al % 128
            xs.append(wj[j] if e == 0 else _cmul(wj[j], small[e]))
        lane = lax.broadcasted_iota(jnp.int32, (8, 128), 1)
        row = lax.broadcasted_iota(jnp.int32, (8, 128), 0)
        diag = (lane & 7) == (7 - row)

        def rev8(v):
            v = pltpu.roll(v, 4, 0)
            v = jnp.where((row & 2) != 0, pltpu.roll(v, 2, 0), pltpu.roll(v, 6, 0))
            return jnp.where((row & 1) != 0, pltpu.roll(v, 1, 0), pltpu.roll(v, 7, 0))

        for g in range(nrows // GRP):
            rs = slice(GRP * g, GRP * (g + 1))
            l8r = (rev8(lam8[0][rs]), rev8(lam8[1][rs]))
            beta = [(one[0][rs], one[1][rs]), l8r]
            for _ in range(2, _NBETA):
                beta.append(_cmul(beta[-1], l8r))
            lhs = jnp.concatenate(
                [jnp.concatenate([x[0][rs], -x[1][rs]], axis=1) for x in xs], axis=0)
            rhs = jnp.concatenate(
                [jnp.concatenate([y[0], y[1]], axis=1) for y in beta], axis=0)
            o = lax.dot_general(_bf(lhs), _bf(rhs), (((1,), (1,)), ((), ())),
                                preferred_element_type=f32)
            for s in range(_NSLAB):
                tot = None
                for j in range(8):
                    a = 8 * s + j
                    if a >= _NA:
                        break
                    v = jnp.where(diag, o[8 * a:8 * a + 8, :], 0.0)
                    v = pltpu.roll(v, j, 1, stride=1, stride_axis=0)
                    tot = v if tot is None else tot + v
                gt_v[s, pl.ds(pl.multiple_of(row0 + GRP * g, 8), GRP), :] = tot

    KR = 16

    def kgen_body(it, c):
        kgen_rows(pl.multiple_of(it * KR, KR), KR)
        return c

    lax.fori_loop(0, D // KR, kgen_body, 0)

    copies[0].wait()
    for m in range(NB):
        tot = None
        for idx, (pm, s) in enumerate(_PLAN):
            if pm != m:
                continue
            v = lax.dot_general(fsel_v[idx], _bf(gt_v[s]), (((1,), (1,)), ((), ())),
                                preferred_element_type=f32)
            tot = v if tot is None else tot + v
        kf_v[m] = tot

    for c in copies[1:]:
        c.wait()

    dskip = dskip_ref[...].astype(f32)

    def out_copy(i):
        r0 = pl.multiple_of(i * T, T)
        return pltpu.make_async_copy(out_v.at[pl.ds(r0, T)], out_hbm.at[pl.ds(r0, T)],
                                     out_sems.at[i])

    def block_body(i, carry):
        r0 = pl.multiple_of(i * T, T)
        xe = u_v[pl.ds(r0, T + 2 * PAD), :].astype(f32)[8:T + 24]
        xne = _bf(_ln(xe))
        xne32 = xne.astype(f32)
        x = xe[8:8 + T]
        xn = xne[8:8 + T]
        xn32 = xne32[8:8 + T]

        uf_v[i] = jnp.dot(ffwd_ref[...], xn, preferred_element_type=f32)

        h = _gelu(_bf(jnp.dot(_bf(_ln(xne32)), w1_v[...],
                              preferred_element_type=f32)).astype(f32))
        h = _bf(h).astype(f32)
        c = D // 4
        hsft = jnp.concatenate([h[7:7 + T, 0:c], h[9:9 + T, c:2 * c],
                                h[6:6 + T, 2 * c:3 * c], h[10:10 + T, 3 * c:]], axis=1)
        hs = _bf(jnp.dot(_bf(hsft), w2_v[...], preferred_element_type=f32)).astype(f32)
        x1 = _bf(xn32 + hs).astype(f32)
        h3 = _gelu(_bf(jnp.dot(_bf(_ln(x1)), w3_v[...],
                               preferred_element_type=f32)).astype(f32))
        h2 = _bf(jnp.dot(_bf(h3), w4_v[...], preferred_element_type=f32)).astype(f32)
        bo = _bf(x1 + h2).astype(f32)
        gate = _bf(bo * jax.nn.sigmoid(bo)).astype(f32)

        acc_v[...] = jnp.zeros((2 * T, D), f32)

        def mac(m, cc):
            kr = kf_v[m, pl.ds(0, T), :]
            ki = kf_v[m, pl.ds(T, T), :]
            ur = uf_v[i - m, pl.ds(0, T), :]
            ui = uf_v[i - m, pl.ds(T, T), :]
            acc_v[pl.ds(0, T), :] += kr * ur - ki * ui
            acc_v[pl.ds(T, T), :] += kr * ui + ki * ur
            return cc

        lax.fori_loop(0, i + 1, mac, 0)
        y = _bf(jnp.dot(finv_ref[...], _bf(acc_v[...]),
                        preferred_element_type=f32)).astype(f32)
        s = _bf(y + _bf(xn32 * dskip).astype(f32)).astype(f32)
        out_v[pl.ds(r0, T), :] = _bf(x + _bf(s * gate).astype(f32))
        out_copy(i).start()
        return carry

    lax.fori_loop(0, NB, block_body, 0)
    for i in range(NB):
        out_copy(i).wait()


@jax.jit
def pallas_recurrent_scan__ssm_conv_s4__mixer_s_mlp__prompt_kernel(
    A_u, A_A_re, A_A_im, A_B_re, A_B_im, A_C_re, A_C_im, A_log_dt, A_Dskip,
    B_x, B_w1, B_w2, B_w3, B_w4,
):
    bf = jnp.bfloat16
    f32 = jnp.float32
    vmem = pl.BlockSpec(memory_space=pltpu.VMEM)
    hbm = pl.BlockSpec(memory_space=pl.ANY)
    out = pl.pallas_call(
        _kernel,
        out_shape=jax.ShapeDtypeStruct((L, D), bf),
        in_specs=[hbm, vmem, vmem, vmem, vmem, vmem, vmem, vmem, vmem,
                  hbm, hbm, hbm, hbm, vmem, vmem, hbm],
        out_specs=hbm,
        scratch_shapes=[
            pltpu.VMEM((L + 2 * PAD, D), bf),
            pltpu.VMEM((D, D), bf),
            pltpu.VMEM((D, D), bf),
            pltpu.VMEM((D, F), bf),
            pltpu.VMEM((F, D), bf),
            pltpu.VMEM((_NSEL, 2 * T, 128), bf),
            pltpu.VMEM((_NSLAB, D, 128), f32),
            pltpu.VMEM((NB, 2 * T, D), f32),
            pltpu.VMEM((NB, 2 * T, D), f32),
            pltpu.VMEM((2 * T, D), f32),
            pltpu.VMEM((L, D), bf),
            pltpu.SemaphoreType.DMA((6,)),
            pltpu.SemaphoreType.DMA((NB,)),
        ],
        compiler_params=pltpu.CompilerParams(vmem_limit_bytes=100 * 1024 * 1024),
    )(A_u.reshape(L, D), A_A_re, A_A_im, A_B_re, A_B_im, A_C_re, A_C_im,
      A_log_dt.reshape(D, 1), A_Dskip.reshape(1, D), B_w1, B_w2, B_w3, B_w4,
      jnp.asarray(_FFWD, dtype=bf), jnp.asarray(_FINV, dtype=bf),
      jnp.asarray(_FSEL, dtype=bf))
    return out.reshape(1, L, D)
```

```python
import numpy as np
import jax
import jax.numpy as jnp
from jax import lax
import jax.experimental.pallas as pl
import jax.experimental.pallas.tpu as pltpu

L = 2048
D = 512
N = 128
F = 1376
T = 128
NB = L // T
EPS = 1e-5
KR = 256
GRP = 8
FCHUNKS = ((0, 512), (512, 1024), (1024, F))

_ALPHA = (
    [j for j in range(8)]
    + [128 + j for j in range(8)]
    + [256 + 2 * j for j in range(4)] + [384 + 2 * j for j in range(4)]
    + [512 + 128 * i + e for i in range(4) for e in (0, 4)]
    + [1024 + 128 * j for j in range(8)]
    + [2048]
)
_NA = len(_ALPHA)
_NSLAB = 6
_NBETA = 16


def _build_tables():
    r_of_l = np.arange(L, dtype=np.float32).astype(jnp.bfloat16).astype(np.int64)
    pos = {}
    for a, al in enumerate(_ALPHA):
        for b in range(_NBETA):
            pos.setdefault(al + 8 * b, (a // 8, (8 * b + a % 8 + 7) % 128))
    k = np.arange(T, dtype=np.float64)
    theta = np.pi * (2 * k + 1) / (2 * T)
    ll = np.arange(T, dtype=np.float64)
    zc = np.exp(-1j * theta[:, None] * ll[None, :])
    ffwd = np.concatenate([zc.real, zc.imag], axis=0)
    finv = np.concatenate([np.cos(theta[None, :] * ll[:, None]),
                           -np.sin(theta[None, :] * ll[:, None])], axis=1) / T
    mats, plan, bnd = [], [], []
    for m in range(NB):
        main_slab = pos[int(r_of_l[T * m])][0]
        acc = np.zeros((T, 128), dtype=np.complex128)
        extra = {}
        for l in range(T):
            sl, lane = pos[int(r_of_l[T * m + l])]
            if sl == main_slab:
                acc[:, lane] += zc[:, l]
            else:
                extra[(sl, lane)] = extra.get((sl, lane), 0) + zc[:, l]
        assert len(extra) <= 1
        plan.append((main_slab, tuple(extra.keys())))
        mats.append(np.concatenate([acc.real, acc.imag], axis=0))
        for v in extra.values():
            bnd.append(np.concatenate([v.real, v.imag]))
    kk = np.arange(T)
    perm = np.empty(2 * T, dtype=np.int64)
    perm[16 * (kk // 8) + kk % 8] = kk
    perm[16 * (kk // 8) + 8 + kk % 8] = T + kk
    bnd = np.stack(bnd)[:, perm]
    bnd = np.broadcast_to(bnd[:, :, None], bnd.shape + (128,))
    return (ffwd[perm].astype(np.float32), finv[:, perm].astype(np.float32),
            np.stack(mats)[:, perm].astype(np.float32),
            np.ascontiguousarray(bnd).astype(np.float32), tuple(plan))


_FFWD, _FINV, _FSEL, _FBND, _PLAN = _build_tables()
_NSEL = len(_PLAN)


_PROFILE = False


class _NullScope:
    def __enter__(self):
        return self

    def __exit__(self, *a):
        return False


def _scope(name):
    return jax.named_scope(name) if _PROFILE else _NullScope()


def _cmul(a, b):
    return (a[0] * b[0] - a[1] * b[1], a[0] * b[1] + a[1] * b[0])


def _ln(x):
    m = jnp.mean(x, axis=-1, keepdims=True)
    xc = x - m
    v = jnp.mean(xc * xc, axis=-1, keepdims=True)
    return xc * lax.rsqrt(v + EPS)


def _gelu(x):
    return x * (0.5 + 0.5 * jnp.tanh(x * (0.7978845608028654 + 0.035677408136300125 * (x * x))))


def _token(v):
    return jnp.where(jnp.abs(v) < 0.0, 1.0, 0.0).astype(jnp.float32)


def _bf(x):
    return x.astype(jnp.bfloat16)


def _kernel(u_hbm, are_hbm, aim_hbm, bre_hbm, bim_hbm, cre_hbm, cim_hbm,
            ldt_hbm, dskip_hbm, w1_hbm, w2_hbm, w3_hbm, w4_hbm,
            ffwd_hbm, finv_hbm, fbnd_hbm, fsel_hbm,
            out_hbm,
            par_v, ldt_ref, dskip_ref, ffwd_ref, finv_ref, fbnd_ref,
            u_v, xn_v, dt_v, w1_v, w2_v, w3_v, w4_v, fsel_v, gt_v, kf_v, uf_v, acc_v,
            out_v, par_sems, in_sems, out_sems):
    assert D // KR == 2
    f32 = jnp.float32
    are_ref, aim_ref, bre_ref, bim_ref, cre_ref, cim_ref = [par_v.at[i] for i in range(6)]
    par_hbm = (are_hbm, aim_hbm, bre_hbm, bim_hbm, cre_hbm, cim_hbm)

    def par_copy(i, it):
        rows = pl.ds(pl.multiple_of(it * KR, KR), KR)
        return pltpu.make_async_copy(par_hbm[i].at[rows], par_v.at[i, rows],
                                     par_sems.at[it * 6 + i])

    small = [
        pltpu.make_async_copy(ldt_hbm, ldt_ref, in_sems.at[6]),
        pltpu.make_async_copy(dskip_hbm, dskip_ref, in_sems.at[7]),
    ]
    copies = [
        pltpu.make_async_copy(fsel_hbm, fsel_v, in_sems.at[0]),
        pltpu.make_async_copy(u_hbm, u_v, in_sems.at[1]),
        pltpu.make_async_copy(w1_hbm, w1_v, in_sems.at[2]),
        pltpu.make_async_copy(w2_hbm, w2_v, in_sems.at[3]),
        pltpu.make_async_copy(w3_hbm, w3_v, in_sems.at[4]),
        pltpu.make_async_copy(w4_hbm, w4_v, in_sems.at[5]),
        pltpu.make_async_copy(ffwd_hbm, ffwd_ref, in_sems.at[8]),
        pltpu.make_async_copy(finv_hbm, finv_ref, in_sems.at[9]),
        pltpu.make_async_copy(fbnd_hbm, fbnd_ref, in_sems.at[10]),
    ]
    small[0].start()
    for it in range(D // KR):
        for i in range(6):
            par_copy(i, it).start()
    small[1].start()
    small[0].wait()
    small[1].wait()
    for i in range(6):
        par_copy(i, 0).wait()
    for c in copies[0:2] + copies[6:]:
        c.start()

    dt_row = jnp.exp(ldt_ref[...].astype(f32)).astype(jnp.bfloat16).astype(f32)
    dt_v[...] = jnp.broadcast_to(dt_row.reshape(1, D), (N, D)).T

    def kgen_rows(row0, nrows):
        sl = pl.ds(row0, nrows)
        dt = dt_v[sl, :]
        lr = dt * are_ref[sl, :].astype(f32)
        li = dt * aim_ref[sl, :].astype(f32)
        mag = jnp.exp(lr)
        lam = (mag * jnp.cos(li), mag * jnp.sin(li))
        db = (dt * bre_ref[sl, :].astype(f32), dt * bim_ref[sl, :].astype(f32))
        w = _cmul((cre_ref[sl, :].astype(f32), cim_ref[sl, :].astype(f32)), db)
        one = (jnp.ones_like(lr), jnp.zeros_like(lr))
        small = [one, lam]
        for _ in range(2, 9):
            small.append(_cmul(small[-1], lam))
        lam8 = small[8]
        lam128 = lam8
        for _ in range(4):
            lam128 = _cmul(lam128, lam128)
        wj = [w]
        for _ in range(1, 17):
            wj.append(_cmul(wj[-1], lam128))
        xs = []
        for al in _ALPHA:
            j, e = al // 128, al % 128
            xs.append(wj[j] if e == 0 else _cmul(wj[j], small[e]))
        lane = lax.broadcasted_iota(jnp.int32, (8, 128), 1)
        row = lax.broadcasted_iota(jnp.int32, (8, 128), 0)

        def rev8(v):
            v = pltpu.roll(v, 4, 0)
            v = jnp.where((row & 2) != 0, pltpu.roll(v, 2, 0), pltpu.roll(v, 6, 0))
            return jnp.where((row & 1) != 0, pltpu.roll(v, 1, 0), pltpu.roll(v, 7, 0))

        for g in range(nrows // GRP):
            rs = slice(GRP * g, GRP * (g + 1))
            l8r = (rev8(lam8[0][rs]), -rev8(lam8[1][rs]))
            beta = [(one[0][rs], one[1][rs]), l8r]
            for _ in range(2, _NBETA):
                beta.append(_cmul(beta[-1], l8r))
            lhs = jnp.concatenate(
                [jnp.concatenate([x[0][rs], x[1][rs]], axis=1) for x in xs], axis=0)
            rhs = jnp.concatenate(
                [jnp.concatenate([y[0], y[1]], axis=1) for y in beta], axis=0)
            o = lax.dot_general(_bf(lhs), _bf(rhs), (((1,), (1,)), ((), ())),
                                preferred_element_type=f32)
            for s in range(_NSLAB):
                tot = jnp.zeros((8, 128), f32)
                for j in range(8):
                    a = 8 * s + j
                    if a >= _NA:
                        break
                    v = pltpu.roll(o[8 * a:8 * a + 8, :], j, 1, stride=1, stride_axis=0)
                    tot = jnp.where((lane & 7) == (7 + j) % 8, v, tot)
                gt_v[s, pl.ds(row0 + GRP * g, GRP), :] = tot


    def kgen_body(it, c):
        @pl.when(it > 0)
        def _():
            for i in range(6):
                par_copy(i, it).wait()
            for c in copies[2:6]:
                c.start()

        kgen_rows(pl.multiple_of(it * KR, KR), KR)
        return c

    with _scope("kgen"):
        lax.fori_loop(0, D // KR, kgen_body, 0)

    for c in copies[0:2] + copies[6:]:
        c.wait()
    with _scope("kdft"):
        sgn = jnp.where((lax.broadcasted_iota(jnp.int32, (1, 8, D), 1) & 1) == 0, 1.0, -1.0)
        prev = None
        nb_used = 0
        for m in range(NB):
            main_slab, extra = _PLAN[m]
            cur = lax.dot_general(fsel_v[m], _bf(gt_v[main_slab]), (((1,), (1,)), ((), ())),
                                  preferred_element_type=f32)
            for (sl, lane_) in extra:
                grow = gt_v[sl].T[lane_:lane_ + 1, :]
                cur = cur + jnp.tile(fbnd_ref[nb_used], (1, D // 128)) * grow
                nb_used += 1
            cur = cur.reshape(T // 8, 2, 8, D)
            if prev is None:
                kf_v[m] = cur.reshape(2 * T, D)
            else:
                re = cur[:, 0] - sgn * prev[:, 1]
                im = cur[:, 1] + sgn * prev[:, 0]
                kf_v[m] = jnp.stack([re, im], axis=1).reshape(2 * T, D)
            prev = cur
            xn = _bf(_ln(u_v[pl.ds(m * T, T), :].astype(f32)))
            xn_v[pl.ds(m * T, T), :] = xn
            uf_v[m] = jnp.dot(ffwd_ref[...], xn, preferred_element_type=f32)

    with _scope("wait_in"):
        for c in copies[2:6]:
            c.wait()

    dskip = dskip_ref[...].astype(f32).reshape(1, D)

    def out_copy(i):
        r0 = i * T
        return pltpu.make_async_copy(out_v.at[pl.ds(r0, T)], out_hbm.at[pl.ds(r0, T)],
                                     out_sems.at[i])

    with _scope("main"):
        def mac_unit(u, dep):
            rows = pl.ds((u >> 2) * 16, 16)
            lanes = pl.ds((u & 3) * 128, 128)
            for blk in range(NB):
                for m in range(blk + 1):
                    kv = kf_v[m, rows, lanes]
                    uv = uf_v[blk - m, rows, lanes]
                    kr, ki, ur, ui = kv[0:8], kv[8:16], uv[0:8], uv[8:16]
                    if m == 0:
                        if dep is not None:
                            kr = kr + dep
                            ki = ki + dep
                        ar = kr * ur - ki * ui
                        ai = kr * ui + ki * ur
                    else:
                        ar = (ar + kr * ur) - ki * ui
                        ai = (ai + kr * ui) + ki * ur
                acc_v[blk, rows, lanes] = jnp.concatenate([ar, ai], axis=0)
                dep = _token(ar + ai)
            return dep

        tok = None
        for u in range(4 * (T // 8)):
            tok = mac_unit(u, tok)

        xn32 = xn_v[...].astype(f32)
        h = _gelu(jnp.dot(_bf(_ln(xn32)), w1_v[...], preferred_element_type=f32))
        zpad = jnp.zeros((8, D), f32)
        hp = jnp.concatenate([zpad, h, zpad], axis=0)
        c = D // 4
        hsft = jnp.concatenate(
            [hp[7:7 + L, 0:c], hp[9:9 + L, c:2 * c],
             hp[6:6 + L, 2 * c:3 * c], hp[10:10 + L, 3 * c:]], axis=1)
        x1 = xn32 + jnp.dot(_bf(hsft), w2_v[...], preferred_element_type=f32)

        z3 = _bf(_ln(x1))
        h2 = None
        for (f0, f1) in FCHUNKS:
            h3 = lax.dot_general(z3, w3_v[f0:f1, :], (((1,), (1,)), ((), ())),
                                 preferred_element_type=f32)
            part = jnp.dot(_bf(_gelu(h3)), w4_v[f0:f1, :], preferred_element_type=f32)
            h2 = part if h2 is None else h2 + part
        bo = x1 + h2
        gate = bo * (0.5 + 0.5 * jnp.tanh(0.5 * bo))

        for b in range(NB):
            rows = slice(b * T, (b + 1) * T)
            y = jnp.dot(finv_ref[...], _bf(acc_v[b]), preferred_element_type=f32)
            sv = y + xn32[rows] * dskip
            x = u_v[pl.ds(b * T, T), :].astype(f32)
            out_v[pl.ds(b * T, T), :] = _bf(x + sv * gate[rows])
            out_copy(b).start()

    for i in range(NB):
        out_copy(i).wait()


@jax.jit
def pallas_recurrent_scan__ssm_conv_s4__mixer_s_mlp__prompt_kernel(
    A_u, A_A_re, A_A_im, A_B_re, A_B_im, A_C_re, A_C_im, A_log_dt, A_Dskip,
    B_x, B_w1, B_w2, B_w3, B_w4,
):
    bf = jnp.bfloat16
    f32 = jnp.float32
    hbm = pl.BlockSpec(memory_space=pltpu.MemorySpace.HBM)
    out = pl.pallas_call(
        _kernel,
        out_shape=jax.ShapeDtypeStruct((L, D), bf),
        in_specs=[hbm] * 17,
        out_specs=hbm,
        scratch_shapes=[
            pltpu.VMEM((6, D, N), bf),
            pltpu.VMEM((D,), bf),
            pltpu.VMEM((D,), bf),
            pltpu.VMEM(_FFWD.shape, bf),
            pltpu.VMEM(_FINV.shape, bf),
            pltpu.VMEM(_FBND.shape, f32),
            pltpu.VMEM((L, D), bf),
            pltpu.VMEM((L, D), bf),
            pltpu.VMEM((D, N), f32),
            pltpu.VMEM((D, D), bf),
            pltpu.VMEM((D, D), bf),
            pltpu.VMEM((F, D), bf),
            pltpu.VMEM((F, D), bf),
            pltpu.VMEM((_NSEL, 2 * T, 128), bf),
            pltpu.VMEM((_NSLAB, D, 128), f32),
            pltpu.VMEM((NB, 2 * T, D), f32),
            pltpu.VMEM((NB, 2 * T, D), f32),
            pltpu.VMEM((NB, 2 * T, D), f32),
            pltpu.VMEM((L, D), bf),
            pltpu.SemaphoreType.DMA((6 * (D // KR),)),
            pltpu.SemaphoreType.DMA((11,)),
            pltpu.SemaphoreType.DMA((NB,)),
        ],
        compiler_params=pltpu.CompilerParams(vmem_limit_bytes=100 * 1024 * 1024),
    )(A_u.reshape(L, D), A_A_re, A_A_im, A_B_re, A_B_im, A_C_re, A_C_im,
      A_log_dt, A_Dskip, B_w1, B_w2, B_w3.T, B_w4,
      jnp.asarray(_FFWD, dtype=bf), jnp.asarray(_FINV, dtype=bf),
      jnp.asarray(_FBND, dtype=f32),
      jnp.asarray(_FSEL, dtype=bf))
    return out.reshape(1, L, D)
```
